```python
import os as _os
_os.environ.setdefault("JAX_PLATFORMS", "cpu")
import jax
import jax.numpy as jnp

def _softmax(x, axis=-1):
    return jax.nn.softmax(x, axis=axis)
def _gelu(x):
    return jax.nn.gelu(x, approximate=True)
def _silu(x):
    return jax.nn.silu(x)
def _sigmoid(x):
    return jax.nn.sigmoid(x)
def _layernorm(x, axis=-1, eps=1e-5):
    m = jnp.mean(x, axis=axis, keepdims=True)
    v = jnp.var(x, axis=axis, keepdims=True)
    return (x - m) / jnp.sqrt(v + eps)
def _scatter_add(tgt, idx, src, axis=0):
    return tgt.at[idx].add(src)
def _segment_sum(src, seg, n):
    return jax.ops.segment_sum(src, seg, n)
class _Rng:
    def __init__(self, key):
        self._k = key
    def _next(self):
        self._k, sub = jax.random.split(self._k)
        return sub
    def normal(self, shape):
        return jax.random.normal(self._next(), shape, dtype=jnp.bfloat16)
    def randint(self, lo, hi, shape):
        return jax.random.randint(self._next(), shape, lo, hi, dtype=jnp.int32)
    def uniform(self, shape, lo=0.0, hi=1.0):
        return jax.random.uniform(self._next(), shape, jnp.bfloat16, lo, hi)
    def permutation(self, n):
        return jax.random.permutation(self._next(), n)


kernel_name = 'concat_heads__sliding_block__sliding_block__prompt'

def setup_inputs():
    _rng = _Rng(jax.random.key(int.from_bytes(__import__("os").urandom(4), "little")))
    _w = (lambda a: (lambda t: t.astype(jnp.bfloat16) if jnp.issubdtype(t.dtype, jnp.floating) else t)(jnp.asarray(a)))
    def _A_setup():
        B, S, D = 1, 2048, 448
        return {
            "x": _w((lambda *s: _rng.normal(s) * 0.2)(B, S, D)),
            "wqkv": _w((lambda *s: _rng.normal(s) * 0.2)(D, 3 * D)),
            "wo": _w((lambda *s: _rng.normal(s) * 0.05)(D, D)),
        }
    _A_in = _A_setup()

    def _B_setup():
        B, S, D = 1, 2048, 448
        return {
            "x": _w((lambda *s: _rng.normal(s) * 0.2)(B, S, D)),
            "wqkv": _w((lambda *s: _rng.normal(s) * 0.2)(D, 3 * D)),
            "wo": _w((lambda *s: _rng.normal(s) * 0.05)(D, D)),
        }
    _B_in = _B_setup()

    return {
        "A_x": _A_in["x"],
        "A_wqkv": _A_in["wqkv"],
        "A_wo": _A_in["wo"],
        "B_x": _B_in["x"],
        "B_wqkv": _B_in["wqkv"],
        "B_wo": _B_in["wo"],
    }

def reference(A_x, A_wqkv, A_wo, B_x, B_wqkv, B_wo):
    def _A_ref(x, wqkv, wo):
        B, S, D = x.shape
        H = 16; Dh = D // H; W = 256
        qkv = (lambda x, *d: x.transpose(*d))((x @ wqkv).reshape(B, S, 3, H, Dh), 2, 0, 3, 1, 4)
        q, k, v = qkv[0], qkv[1], qkv[2]
        scores = jnp.einsum("bhqd,bhkd->bhqk", q, k) * (Dh ** -0.5)
        idx = jnp.arange(S)
        mask = (idx[:, None] - idx[None, :] >= 0) & (idx[:, None] - idx[None, :] < W)
        scores = jnp.where(mask[None, None], scores, -1e9)
        p = _softmax(scores, axis=-1)
        o = jnp.einsum("bhqk,bhkd->bhqd", p, v)
        return (lambda x, *d: x.transpose(*d))(o, 0, 2, 1, 3).reshape(B, S, D) @ wo

    def _B_ref(x, wqkv, wo):
        B, S, D = x.shape
        H = 16; Dh = D // H; W = 256
        qkv = (lambda x, *d: x.transpose(*d))((x @ wqkv).reshape(B, S, 3, H, Dh), 2, 0, 3, 1, 4)
        q, k, v = qkv[0], qkv[1], qkv[2]
        scores = jnp.einsum("bhqd,bhkd->bhqk", q, k) * (Dh ** -0.5)
        idx = jnp.arange(S)
        mask = (idx[:, None] - idx[None, :] >= 0) & (idx[:, None] - idx[None, :] < W)
        scores = jnp.where(mask[None, None], scores, -1e9)
        p = _softmax(scores, axis=-1)
        o = jnp.einsum("bhqk,bhkd->bhqd", p, v)
        return (lambda x, *d: x.transpose(*d))(o, 0, 2, 1, 3).reshape(B, S, D) @ wo

    a = _A_ref(A_x, A_wqkv, A_wo)
    b = _B_ref(B_x, B_wqkv, B_wo)
    return jnp.concatenate([a, b], axis=-1)
```

```python
import functools
import math

import jax
import jax.numpy as jnp
from jax import lax
from jax.experimental import pallas as pl
from jax.experimental.pallas import tpu as pltpu

S = 2048
D = 448
H = 16
DH = 28
G = 4
GW = 112
QB = 128
NQ = S // QB
HD = D // 2
HG = GW // 2
HQ = QB // 2
NEG = -1e30
QSCALE = (DH ** -0.5) * math.log2(math.e)

F32 = jnp.float32
BF16 = jnp.bfloat16
U32 = jnp.uint32

WCH = ((384, 512), (0, 384), (896, 448))
XCH = 256
NX = S // XCH
CA = 384
L0 = 3
PB = 6
NIT = (NQ - 1 - L0) // PB


def _pack(x):
    return pltpu.bitcast(x.astype(BF16), U32)


def _bf(x):
    return pltpu.bitcast(x, BF16)


def _cat(xs, axis=0):
    return xs[0] if len(xs) == 1 else jnp.concatenate(xs, axis=axis)


class _Refs:
    pass


def _zero_of(c, x):
    parts = [x[r:r + 8, l:l + QB] for r in range(0, x.shape[0], 8) for l in range(0, x.shape[1], QB)]
    return functools.reduce(lambda u, v: u | v, parts) & c.pm[0, 0] & c.pm[2, 0]


def _scores(c, b, q, g, deps=()):
    qg = c.qt[b, q % 2, g * HG:(g + 1) * HG, :]
    zero8 = jnp.zeros((8, QB), U32)
    if deps:
        z = functools.reduce(lambda u, v: u | v, deps)
        qg = _cat([qg[0:HG - 8], qg[HG - 8:] | z])

    def wmat(t, s):
        if t:
            return _bf(_cat([qg & c.wm[t, s], zero8]))
        rows, run = [], []
        for n in range(HG // 8 + 1):
            if {(16 * n) // DH, (16 * n + 15) // DH} & {s, s ^ 2}:
                run.append(n)
                continue
            if run:
                lo, hi = 8 * run[0], 8 * run[-1] + 8
                rows.append(qg[lo:hi] & c.wm[0, s, lo:hi])
            rows.append(zero8)
            run = []
        return _bf(_cat(rows))

    @functools.lru_cache(None)
    def krows(v, lo, hi):
        parts = []
        for blk in range((4 + lo) // 8, (4 + hi - 1) // 8 + 1):
            n0 = max(4 + lo - 8 * blk, 0)
            n1 = min(4 + hi - 8 * blk, 8)
            parts.append(c.ks[b, (q + blk) % PB, g, v, 8 * n0:8 * n1, :])
        return _cat(parts)

    def mm(rows, w):
        return jnp.dot(_bf(rows), w, preferred_element_type=F32)

    def mixed(t):
        res = []
        for s in range(4):
            hi, lo = krows(s // 2, t, t + 1), krows(s // 2, t - 17, t - 16)
            row = lax.select(c.hodd, lo, hi) if s % 2 else lax.select(c.hodd, hi, lo)
            res.append(mm(row, wmat(t, s)))
        return res

    chunks = []
    if q >= 2:
        mix = {}
        for t in (1, 2, 0, 3):
            if t == 0:
                com = [mm(krows(s // 2, -13, 1), wmat(0, s)) for s in range(4)]
            else:
                mix[t] = mixed(t)
        for s in range(4):
            ch = {k - 13: com[s][16 * k:16 * k + 16] for k in range(14)}
            hi = [ch.pop(0)] + [mix[t][s ^ 1] for t in (1, 2, 3)]
            lo = [mix[t][s] for t in (1, 2, 3)] + [ch.pop(-13)]
            for k in range(4):
                ch[k] = lax.select(c.tri[k], hi[k], lo[k])
            chunks.append(ch)
    else:
        lo = -4 - 8 * q
        neg = jnp.full((16, QB), NEG, F32)
        for s in range(4):
            sc = mm(krows(s // 2, lo, 4), wmat(0, s))
            ch = {k: sc[16 * (k - lo):16 * (k - lo) + 16] for k in range(lo, 4)}
            for k in range(lo, lo + 4):
                ch[k] = lax.select(c.hi16, ch[k], neg)
            for k in range(4):
                ch[k] = lax.select(c.tri[k], ch[k], neg)
            chunks.append(ch)
    res = []
    for ch in chunks:
        mx = functools.reduce(jnp.maximum, ch.values())
        res.append((ch, jnp.broadcast_to(jnp.max(mx, axis=0, keepdims=True), (8, QB))))
    return res


def _save_scores(c, sc):
    for s, (ch, m) in enumerate(sc):
        c.sv[s] = _cat([ch[k] for k in range(-12, 4)] + [m])


def _load_scores(c):
    return [({k: c.sv[s, 16 * (k + 12):16 * (k + 13)] for k in range(-12, 4)}, c.sv[s, 256:264])
            for s in range(4)]


def _softmax_pv(c, sc, b, q, g):
    t0 = max(2 - q, 0)
    mbits = [pltpu.bitcast(m, U32) for _, m in sc]
    mcur = [_cat([m, m]) for _, m in sc]
    pm = functools.lru_cache(None)(lambda i, k: c.pm[i, k])

    @functools.lru_cache(None)
    def P(s, k):
        p = jnp.exp2(sc[s][0][k] - mcur[s])
        p = pltpu.bitcast(p, U32)
        return (p[8:16] & jnp.uint32(0xFFFF0000)) | (p[0:8] >> 16)

    def pt_chunk(h, n):
        if n < 4:
            return P(h, n) & pm(0, n)
        if n >= 20:
            return P(h ^ 2, n - 20) & pm(3, n - 20)
        x = lax.select(c.hi, P(h ^ 2, n - 4 if n < 8 else n - 20), P(h, n - 16))
        if n < 8:
            return x & pm(1, n - 4)
        return x & pm(2, n - 16) if n >= 16 else x

    acc = [None] * 4
    for t in range(2, t0 - 1, -1):
        dt = [[None] * 8 for _ in range(4)]
        for n in range(8 * t + 7, 8 * t - 1, -1):
            for h in range(4):
                dt[h][n - 8 * t] = pt_chunk(h, n)
            if n % 2 == 0 and n > max(8, 8 * t0):
                for s in range(4):
                    z = dt[s ^ 3][n + 1 - 8 * t] >> 31
                    m = pltpu.bitcast(mbits[s] | (z + z), F32)
                    mcur[s] = _cat([m, m])
        for h in range(4):
            head = g * 4 + h
            vt = _bf(c.vt[b, (q - 2 + t) % PB, head * 16:(head + 1) * 16, :])
            o = jnp.dot(vt, _bf(_cat(dt[h])), preferred_element_type=F32)
            acc[h] = o if acc[h] is None else o + acc[h]
    outs = []
    for h in range(4):
        o = acc[h]
        l = o[28:29] if h % 2 == 0 else o[0:1]
        r = pl.reciprocal(l, approx=True)
        r = r * (2.0 - l * r)
        outs.append(o * r)
    res = []
    for p in range(2):
        e, o = outs[2 * p], outs[2 * p + 1]
        res += [e[0:24], lax.select(c.low4, e[24:32], o[0:8]), o[8:32]]
    c.ot[b, q % PB, g * HG:(g + 1) * HG, :] = _pack(_cat(res))


def _proj(c, b, q, off, part):
    x = c.xv[b, q // 2 + off // 2, :, (q % 2) * QB:(q % 2 + 1) * QB]
    return jnp.dot(_bf(c.wt[b, part * HD:(part + 1) * HD, :]), x, preferred_element_type=F32)


def _prep_k(c, b, q, kT):
    zpad = jnp.zeros((16, QB), F32)
    last = []
    slabs = _cat([x for g in range(G) for x in (kT[g * GW:(g + 1) * GW], zpad)])
    kp = pltpu.bitcast(slabs.astype(BF16).T, U32)
    for g in range(G):
        w = kp[:, g * QB:(g + 1) * QB]
        ev = pltpu.bitcast(w << 16, F32)
        od = pltpu.bitcast(w & jnp.uint32(0xFFFF0000), F32)
        knew = _pack(_cat([v[8 * n:8 * n + 8] for n in range(8) for v in (ev, od)]))
        prev = jnp.zeros((32, QB), U32) if q == 0 else c.kr[b, g]
        c.kr[b, g] = knew[32:]
        lag = _cat([prev, knew[0:32]])
        c.ks[b, q % PB, g, 0] = lax.select(c.hhi, knew, lag)
        c.ks[b, q % PB, g, 1] = lax.select(c.hhi, lag, knew)
        last.append(knew[HQ - 8:])
    return _cat(last)


def _store_v(c, b, q, vT):
    rows = []
    for p in range(H // 2):
        base = 56 * p
        mid = vT[base + 24:base + 32]
        rows += [vT[base:base + 24], lax.select(c.low4, mid, c.ones),
                 lax.select(c.low4, c.ones, mid), vT[base + 32:base + 56]]
    c.vt[b, q % PB] = _pack(_cat(rows))


def _unit(b, q, fill, extra=(), sync=(), at=0):
    r = []
    for g in range(G):
        r += [("QK", b, q, g)] + (list(sync) if g == at else []) + [fill[g], ("AV", b, q, g)]
        if g < len(extra) and extra[g]:
            r.append(extra[g])
    return r


def _steady(b, q):
    return _unit(b, q, [("O", b, q - 1), ("K", b, q + 1), ("Q", b, q + 1), ("V", b, q + 1)])


def _programs():
    A, B = 0, 1
    KC, QC, VC = WCH
    pro = [("WAIT", 0), ("TW", A, KC, 0, 256), ("WAIT", 1), ("TW", A, KC, 256, D),
           ("WAIT", 2), ("KM", A, 0), ("KM", A, 1),
           ("WAIT", 3), ("TW", A, QC, 0, D), ("KP", A, 0), ("KP", A, 1), ("K", A, 2),
           ("Q", A, 0), ("Q", A, 1),
           ("WAIT", 4), ("TW", A, VC, 0, D)]
    pro += [("QK", A, 0, g) for g in range(G)] + [("V", A, 0)] + [("AV", A, 0, g) for g in range(G)]
    pro += _unit(A, 1, [("V", A, 1), ("Q", A, 2), ("V", A, 2), ("K", A, 3)])
    sync = [("WAIT", 5)] + [("TW", B, ch, 0, D) for ch in WCH] + [("TO", A), ("TO", B)]
    pro += _unit(A, 2, [("Q", A, 3), ("V", A, 3), ("K", B, 0), ("Q", B, 0)], sync=sync, at=1)
    pro += [("V", B, 0)]
    pro += _unit(B, 0, [("K", B, 1), ("Q", B, 1), ("O", A, 0), ("O", A, 1)])
    pro += _unit(B, 1, [("V", B, 1), ("K", B, 2), ("Q", B, 2), ("V", B, 2)],
                 extra=[None, ("O", B, 0)])
    pro += _steady(B, 2) + [("QKS", A, L0, 0), ("OUT", 0, L0 - 1, 0, 2 * D), ("WAIT", 6)]

    body = []
    for j in range(PB):
        body += _steady(A, L0 + j) + _steady(B, L0 + j)
    body = body[1:] + [("QKS", A, L0 + PB, 0), ("OUT", L0 - 1, PB, 0, 2 * D)]
    body[1] = ("AVL",) + body[1][1:]

    q = NQ - 1
    epi = [("O", A, q - 1), ("AVL", A, q, 0), ("QK", A, q, 1),
           ("O", B, q - 1), ("OUT", q - 1, 1, 0, 2 * D), ("AV", A, q, 1),
           ("QK", A, q, 2), ("QK", A, q, 3), ("AV", A, q, 2), ("QK", B, q, 3), ("AV", A, q, 3),
           ("QK", B, q, 2), ("AV", B, q, 3), ("OA", A, q), ("OUT", q, 1, 0, CA), ("AV", B, q, 2),
           ("QK", B, q, 1), ("QK", B, q, 0), ("AV", B, q, 1), ("OP", B, q, 256, D),
           ("AV", B, q, 0), ("OP", B, q, 128, 256), ("OP", B, q, 0, 128), ("OE", B, q),
           ("OUT", q, 1, CA, 2 * D)]
    return pro, body, epi


def _kernel(xa, wa, woa, xb, wb, wob, out, wv, wov, xv, ob, wt, wot, wm, pm, qt, kr, ks, vt, ot,
            sv, sem):
    c = _Refs()
    c.wt, c.wm, c.pm, c.qt, c.kr, c.ks, c.vt, c.ot, c.xv, c.sv = (
        wt, wm, pm, qt, kr, ks, vt, ot, xv, sv)

    def w_copy(ch, r0=0, r1=D):
        rows, cols = pl.ds(r0, r1 - r0), pl.ds(*ch)
        return wa.at[rows, cols], wv.at[0, rows, cols]

    def x_copy(b, k, lo=0, n=XCH):
        return (xa, xb)[b].at[0, :, pl.ds(k * XCH + lo, n)], xv.at[b, k, :, pl.ds(lo, n)]

    groups = [
        [w_copy(WCH[0], 0, 256)],
        [w_copy(WCH[0], 256, D)],
        [x_copy(0, 0)],
        [x_copy(0, 1, 0, QB), w_copy(WCH[1])],
        [w_copy(WCH[2]), x_copy(0, 1, QB, QB)],
        [(wb, wv.at[1]), x_copy(1, 0), x_copy(1, 1), (woa, wov.at[0]), (wob, wov.at[1])],
        [x_copy(b, k) for k in range(2, NX) for b in range(2)],
    ]
    osem = sem.at[len(groups)]

    def in_copies(n):
        return [pltpu.make_async_copy(src, dst, sem.at[n]) for src, dst in groups[n]]

    def run(prog, it=None):
        off = 0 if it is None else it * PB
        val = {}
        pend = []

        def rows(q, n=1):
            if it is None:
                return pl.ds(q * QB, n * QB)
            return pl.ds(pl.multiple_of((q + off) * QB, QB), n * QB)

        def take_deps():
            ready = [_zero_of(c, x) for n, x in pend if n == 0]
            pend[:] = [(n - 1, x) for n, x in pend if n > 0]
            return ready

        def store_out(q, c0, c1, x):
            x = x.T.astype(BF16)
            ob[rows(q), c0:c1] = x
            pend.append((1, pltpu.bitcast(x[QB - 16:], U32)))

        for item in prog:
            op, a = item[0], item[1:]
            if op == "WAIT":
                for cp in in_copies(a[0]):
                    cp.wait()
            elif op == "TW":
                b, (lo, n), r0, r1 = a
                wt[b, lo // 2:(lo + n) // 2, r0:r1] = pltpu.bitcast(wv[b, r0:r1, lo:lo + n].T, U32)
            elif op == "TO":
                wot[a[0]] = pltpu.bitcast(wov[a[0]].T, U32)
            elif op == "K":
                pend.append((1, _prep_k(c, *a, _proj(c, *a, off, 1))))
            elif op == "KM":
                val["k", a] = _proj(c, *a, off, 1)
            elif op == "KP":
                _prep_k(c, *a, val.pop(("k", a)))
            elif op == "Q":
                qt[a[0], a[1] % 2] = _pack(_proj(c, *a, off, 0) * QSCALE)
            elif op == "V":
                _store_v(c, *a, _proj(c, *a, off, 2))
            elif op == "QK":
                val[a] = _scores(c, *a, take_deps())
            elif op == "QKS":
                _save_scores(c, _scores(c, *a, take_deps()))
            elif op == "AV":
                _softmax_pv(c, val.pop(a), *a)
            elif op == "AVL":
                _softmax_pv(c, _load_scores(c), *a)
            elif op in ("O", "OA"):
                b, q = a
                o = jnp.dot(_bf(wot[b]), _bf(ot[b, q % PB]), preferred_element_type=F32)
                if op == "OA":
                    store_out(q, 0, CA, o[0:CA])
                    val["tail"] = o[CA:]
                elif b == 0:
                    val["o", q] = o
                else:
                    store_out(q, 0, 2 * D, _cat([val.pop(("o", q)), o]))
            elif op == "OP":
                b, q, lo, hi = a
                rhs = _bf(ot[b, q % PB, lo // 2:hi // 2, :])
                cuts = (0, 32, 96, 160, 224) if lo == 0 else (0, 56, 112, 168, 224)
                part = [jnp.dot(_bf(wot[b, r0:r1, lo:hi]), rhs, preferred_element_type=F32)
                        for r0, r1 in zip(cuts, cuts[1:])]
                if "part" in val:
                    prev = _cat(val["part"])
                    part = [x + prev[2 * r0:2 * r1] for x, r0, r1 in zip(part, cuts, cuts[1:])]
                val["part"] = part
            elif op == "OE":
                store_out(a[1], CA, 2 * D, _cat([val.pop("tail")] + val.pop("part")))
            elif op == "OUT":
                r, cols = rows(a[0], a[1]), pl.ds(a[2], a[3] - a[2])
                pltpu.make_async_copy(ob.at[r, cols], out.at[0, r, cols], osem).start()
            else:
                raise ValueError(op)
        assert not val

    for n in range(len(groups)):
        for cp in in_copies(n):
            cp.start()

    def iota(rows, dim):
        return lax.broadcasted_iota(jnp.int32, (rows, QB), dim)

    def bits(mask, word=0xFFFFFFFF):
        return jnp.where(mask, jnp.uint32(word), jnp.uint32(0))

    phead = iota(HG, 0) // (DH // 2)
    sub = iota(HG, 1) // 16
    for t in range(4):
        slot = 2 * (sub // 4) + (jnp.where(sub % 4 >= t, 1, 0) if t else 0)
        for s in range(4):
            wm[t, s] = bits(phead == (slot ^ s))
    lane8, row8 = iota(8, 1), iota(8, 0)
    hib = bits(lane8 >= 64)
    for k in range(4):
        key = 16 * k + 2 * row8
        tb = bits(key <= lane8 % 64, 0xFFFF) | bits(key + 1 <= lane8 % 64, 0xFFFF0000)
        pm[0, k] = ~(tb | hib)
        pm[1, k] = ~(tb & hib)
        pm[2, k] = tb | hib
        pm[3, k] = tb & hib
    lane16, row16 = iota(16, 1), iota(16, 0)
    key16 = 2 * (row16 % 8) + row16 // 8
    c.tri = [16 * k + key16 <= lane16 % 64 for k in range(4)]
    c.hi16 = lane16 >= 64
    c.hi = lane8 >= 64
    c.hodd = (lane8 // DH) % 2 == 1
    c.hhi = iota(HQ, 1) >= 2 * DH
    c.low4 = row8 < 4
    c.ones = jnp.where(row8 % 4 == 0, 1.0, 0.0).astype(F32)

    pro, body, epi = _programs()

    def step(it, carry):
        @pl.when(it == 0)
        def _():
            run(pro)

        run(body, it)

        @pl.when(it == NIT - 1)
        def _():
            run(epi)
            pltpu.make_async_copy(ob, out.at[0], osem).wait()

        return carry

    lax.fori_loop(0, NIT, step, 0)


@jax.jit
def pallas_concat_heads__sliding_block__sliding_block__prompt_kernel(
        A_x, A_wqkv, A_wo, B_x, B_wqkv, B_wo):
    xa = jnp.transpose(A_x, (0, 2, 1))
    xb = jnp.transpose(B_x, (0, 2, 1))
    return pl.pallas_call(
        _kernel,
        in_specs=[pl.BlockSpec(memory_space=pl.ANY)] * 6,
        out_specs=pl.BlockSpec(memory_space=pl.ANY),
        out_shape=jax.ShapeDtypeStruct((1, S, 2 * D), BF16),
        scratch_shapes=[
            pltpu.VMEM((2, D, 3 * D), BF16),
            pltpu.VMEM((2, D, D), BF16),
            pltpu.VMEM((2, NX, D, XCH), BF16),
            pltpu.VMEM((S, 2 * D), BF16),
            pltpu.VMEM((2, 3 * HD, D), U32),
            pltpu.VMEM((2, HD, D), U32),
            pltpu.VMEM((4, 4, HG, QB), U32),
            pltpu.VMEM((4, 4, 8, QB), U32),
            pltpu.VMEM((2, 2, HD, QB), U32),
            pltpu.VMEM((2, G, 32, QB), U32),
            pltpu.VMEM((2, PB, G, 2, HQ, QB), U32),
            pltpu.VMEM((2, PB, H * 16, QB), U32),
            pltpu.VMEM((2, PB, HD, QB), U32),
            pltpu.VMEM((4, 264, QB), F32),
            pltpu.SemaphoreType.DMA((8,)),
        ],
        compiler_params=pltpu.CompilerParams(
            vmem_limit_bytes=64 * 1024 * 1024,
            disable_semaphore_checks=True,
            disable_bounds_checks=True),
        name="swa_fused",
    )(xa, A_wqkv, A_wo, xb, B_wqkv, B_wo)
```

```python
import functools
import math

import jax
import jax.numpy as jnp
from jax import lax
from jax.experimental import pallas as pl
from jax.experimental.pallas import tpu as pltpu

S = 2048
D = 448
H = 16
DH = 28
G = 4
GW = 112
QB = 128
NQ = S // QB
HD = D // 2
HG = GW // 2
HQ = QB // 2
NEG = -1e30
QSCALE = (DH ** -0.5) * math.log2(math.e)

F32 = jnp.float32
BF16 = jnp.bfloat16
U32 = jnp.uint32

WCH = ((384, 512), (0, 384), (896, 448))
XCH = 256
NX = S // XCH
CA = 384
L0 = 3
PB = 6
NIT = (NQ - 1 - L0) // PB


def _pack(x):
    return pltpu.bitcast(x.astype(BF16), U32)


def _bf(x):
    return pltpu.bitcast(x, BF16)


def _cat(xs, axis=0):
    return xs[0] if len(xs) == 1 else jnp.concatenate(xs, axis=axis)


class _Refs:
    pass


def _zero_of(c, x):
    parts = [x[r:r + 8, l:l + QB] for r in range(0, x.shape[0], 8) for l in range(0, x.shape[1], QB)]
    return functools.reduce(lambda u, v: u | v, parts) & c.pm[0, 0, 0:8] & c.pm[2, 0, 0:8]


def _scores(c, b, q, g, deps=()):
    qg = c.qt[b, q % 2, g * HG:(g + 1) * HG, :]
    zero8 = jnp.zeros((8, QB), U32)
    if deps:
        z = functools.reduce(lambda u, v: u | v, deps)
        qg = _cat([qg[0:HG - 8], qg[HG - 8:] | z])

    def wmat(t, s):
        if t:
            return _bf(_cat([qg & c.wm[t, s], zero8]))
        rows, run = [], []
        for n in range(HG // 8 + 1):
            if {(16 * n) // DH, (16 * n + 15) // DH} & {s, s ^ 2}:
                run.append(n)
                continue
            if run:
                lo, hi = 8 * run[0], 8 * run[-1] + 8
                rows.append(qg[lo:hi] & c.wm[0, s, lo:hi])
            rows.append(zero8)
            run = []
        return _bf(_cat(rows))

    @functools.lru_cache(None)
    def krows(v, lo, hi):
        parts = []
        for blk in range((4 + lo) // 8, (4 + hi - 1) // 8 + 1):
            n0 = max(4 + lo - 8 * blk, 0)
            n1 = min(4 + hi - 8 * blk, 8)
            parts.append(c.ks[b, (q + blk) % PB, g, v, 8 * n0:8 * n1, :])
        return _cat(parts)

    def mm(rows, w):
        return jnp.dot(_bf(rows), w, preferred_element_type=F32)

    def mixed(t):
        res = []
        for s in range(4):
            hi, lo = krows(s // 2, t, t + 1), krows(s // 2, t - 17, t - 16)
            row = lax.select(c.hodd, lo, hi) if s % 2 else lax.select(c.hodd, hi, lo)
            res.append(mm(row, wmat(t, s)))
        return res

    scs = []
    if q >= 2:
        mix = {}
        for t in (1, 2, 0, 3):
            if t == 0:
                com = [mm(krows(s // 2, -13, 1), wmat(0, s)) for s in range(4)]
            else:
                mix[t] = mixed(t)
        for s in range(4):
            hi = _cat([com[s][208:224]] + [mix[t][s ^ 1] for t in (1, 2, 3)])
            lo = _cat([mix[t][s] for t in (1, 2, 3)] + [com[s][0:16]])
            scs.append(_cat([com[s][16:208], lax.select(c.tri, hi, lo)]))
    else:
        neg = jnp.full((64, QB), NEG, F32)
        for s in range(4):
            sc = mm(krows(s // 2, -4 - 8 * q, 4), wmat(0, s))
            scs.append(_cat([lax.select(c.hi64, sc[0:64], neg)] + ([sc[64:192]] if q else [])
                            + [lax.select(c.tri, sc[64 + 128 * q:], neg)]))
    res = []
    for sc in scs:
        mx = functools.reduce(jnp.maximum, [sc[r:r + 64] for r in range(0, sc.shape[0], 64)])
        res.append((sc, jnp.broadcast_to(jnp.max(mx, axis=0, keepdims=True), (8, QB))))
    return res


def _save_scores(c, sc):
    for s, (x, m) in enumerate(sc):
        c.sv[s] = _cat([x, m])


def _load_scores(c):
    return [(c.sv[s, 0:256], c.sv[s, 256:264]) for s in range(4)]


def _softmax_pv(c, sc, b, q, g):
    t0 = max(2 - q, 0)
    top = sc[0][0].shape[0] - 64
    mbits = [pltpu.bitcast(m, U32) for _, m in sc]
    mcur = [_cat([m] * 4) for _, m in sc]
    pm = functools.lru_cache(None)(lambda i, k: c.pm[i, k])

    @functools.lru_cache(None)
    def P(s, k):
        p = jnp.exp2(sc[s][0][top + 32 * k:top + 32 * k + 32] - mcur[s])
        p = pltpu.bitcast(p, U32).reshape(2, 16, QB)
        return ((p[:, 8:16] & jnp.uint32(0xFFFF0000)) | (p[:, 0:8] >> 16)).reshape(16, QB)

    def pt_rows(h, n):
        if n < 2:
            return P(h, n) & pm(0, n)
        if n >= 10:
            return P(h ^ 2, n - 10) & pm(3, n - 10)
        x = lax.select(c.hi16, P(h ^ 2, n - 2 if n < 4 else n - 10), P(h, n - 8))
        if n < 4:
            return x & pm(1, n - 2)
        return x & pm(2, n - 8) if n >= 8 else x

    acc = [None] * 4
    for t in range(2, t0 - 1, -1):
        dt = [[None] * 4 for _ in range(4)]
        for n in range(4 * t + 3, 4 * t - 1, -1):
            for h in range(4):
                dt[h][n - 4 * t] = pt_rows(h, n)
            if n > max(4, 4 * t0):
                for s in range(4):
                    z = dt[s ^ 3][n - 4 * t][8:16] >> 31
                    mcur[s] = _cat([pltpu.bitcast(mbits[s] | (z + z), F32)] * 4)
        for h in range(4):
            head = g * 4 + h
            vt = _bf(c.vt[b, (q - 2 + t) % PB, head * 16:(head + 1) * 16, :])
            o = jnp.dot(vt, _bf(_cat(dt[h])), preferred_element_type=F32)
            acc[h] = o if acc[h] is None else o + acc[h]
    outs = []
    for h in range(4):
        o = acc[h]
        l = o[28:29] if h % 2 == 0 else o[0:1]
        r = pl.reciprocal(l, approx=True)
        r = r * (2.0 - l * r)
        outs.append(o * r)
    res = []
    for p in range(2):
        e, o = outs[2 * p], outs[2 * p + 1]
        res += [e[0:24], lax.select(c.low4, e[24:32], o[0:8]), o[8:32]]
    c.ot[b, q % PB, g * HG:(g + 1) * HG, :] = _pack(_cat(res))


def _proj(c, b, q, off, part):
    x = c.xv[b, q // 2 + off // 2, :, (q % 2) * QB:(q % 2 + 1) * QB]
    return jnp.dot(_bf(c.wt[b, part * HD:(part + 1) * HD, :]), x, preferred_element_type=F32)


def _prep_k(c, b, q, kT):
    zpad = jnp.zeros((16, QB), F32)
    last = []
    slabs = _cat([x for g in range(G) for x in (kT[g * GW:(g + 1) * GW], zpad)])
    kp = pltpu.bitcast(slabs.astype(BF16).T, U32)
    for g in range(G):
        w = kp[:, g * QB:(g + 1) * QB]
        ev = pltpu.bitcast(w << 16, F32)
        od = pltpu.bitcast(w & jnp.uint32(0xFFFF0000), F32)
        knew = _pack(_cat([ev.reshape(8, 8, QB), od.reshape(8, 8, QB)], axis=1).reshape(QB, QB))
        prev = jnp.zeros((32, QB), U32) if q == 0 else c.kr[b, g]
        c.kr[b, g] = knew[32:]
        lag = _cat([prev, knew[0:32]])
        c.ks[b, q % PB, g, 0] = lax.select(c.hhi, knew, lag)
        c.ks[b, q % PB, g, 1] = lax.select(c.hhi, lag, knew)
        last.append(knew[HQ - 8:])
    return _cat(last)


def _store_v(c, b, q, vT):
    rows = []
    for p in range(H // 2):
        base = 56 * p
        mid = vT[base + 24:base + 32]
        rows += [vT[base:base + 24], lax.select(c.low4, mid, c.ones),
                 lax.select(c.low4, c.ones, mid), vT[base + 32:base + 56]]
    c.vt[b, q % PB] = _pack(_cat(rows))


def _unit(b, q, fill, extra=(), sync=(), at=0):
    r = []
    for g in range(G):
        r += [("QK", b, q, g)] + (list(sync) if g == at else []) + [fill[g], ("AV", b, q, g)]
        if g < len(extra) and extra[g]:
            r.append(extra[g])
    return r


def _steady(b, q):
    return _unit(b, q, [("O", b, q - 1), ("K", b, q + 1), ("Q", b, q + 1), ("V", b, q + 1)])


def _programs():
    A, B = 0, 1
    KC, QC, VC = WCH
    pro = [("WAIT", 0), ("TW", A, KC, 0, 256), ("WAIT", 1), ("TW", A, KC, 256, D),
           ("WAIT", 2), ("KM", A, 0), ("KM", A, 1),
           ("WAIT", 3), ("TW", A, QC, 0, D), ("KP", A, 0), ("KP", A, 1), ("K", A, 2),
           ("Q", A, 0), ("Q", A, 1),
           ("WAIT", 4), ("TW", A, VC, 0, D)]
    pro += [("QK", A, 0, g) for g in range(G)] + [("V", A, 0)] + [("AV", A, 0, g) for g in range(G)]
    pro += _unit(A, 1, [("V", A, 1), ("Q", A, 2), ("V", A, 2), ("K", A, 3)])
    sync = [("WAIT", 5)] + [("TW", B, ch, 0, D) for ch in WCH] + [("TO", A), ("TO", B)]
    pro += _unit(A, 2, [("Q", A, 3), ("V", A, 3), ("K", B, 0), ("Q", B, 0)], sync=sync, at=1)
    pro += [("V", B, 0)]
    pro += _unit(B, 0, [("K", B, 1), ("Q", B, 1), ("O", A, 0), ("O", A, 1)])
    pro += _unit(B, 1, [("V", B, 1), ("K", B, 2), ("Q", B, 2), ("V", B, 2)],
                 extra=[None, ("O", B, 0)])
    pro += _steady(B, 2) + [("QKS", A, L0, 0), ("OUT", 0, L0 - 1, 0, 2 * D), ("WAIT", 6)]

    body = []
    for j in range(PB):
        body += _steady(A, L0 + j) + _steady(B, L0 + j)
    body = body[1:] + [("QKS", A, L0 + PB, 0), ("OUT", L0 - 1, PB, 0, 2 * D)]
    body[1] = ("AVL",) + body[1][1:]

    q = NQ - 1
    epi = [("O", A, q - 1), ("AVL", A, q, 0), ("QK", A, q, 1),
           ("O", B, q - 1), ("OUT", q - 1, 1, 0, 2 * D), ("AV", A, q, 1),
           ("QK", A, q, 2), ("QK", A, q, 3), ("AV", A, q, 2), ("QK", B, q, 3), ("AV", A, q, 3),
           ("QK", B, q, 2), ("AV", B, q, 3), ("OA", A, q), ("OUT", q, 1, 0, CA), ("AV", B, q, 2),
           ("QK", B, q, 1), ("QK", B, q, 0), ("AV", B, q, 1), ("OP", B, q, 256, D),
           ("AV", B, q, 0), ("OP", B, q, 128, 256), ("OP", B, q, 0, 128), ("OE", B, q),
           ("OUT", q, 1, CA, 2 * D)]
    return pro, body, epi


def _kernel(xa, wa, woa, xb, wb, wob, out, wv, wov, xv, ob, wt, wot, wm, pm, qt, kr, ks, vt, ot,
            sv, sem):
    c = _Refs()
    c.wt, c.wm, c.pm, c.qt, c.kr, c.ks, c.vt, c.ot, c.xv, c.sv = (
        wt, wm, pm, qt, kr, ks, vt, ot, xv, sv)

    def w_copy(ch, r0=0, r1=D):
        rows, cols = pl.ds(r0, r1 - r0), pl.ds(*ch)
        return wa.at[rows, cols], wv.at[0, rows, cols]

    def x_copy(b, k, lo=0, n=XCH):
        return (xa, xb)[b].at[0, :, pl.ds(k * XCH + lo, n)], xv.at[b, k, :, pl.ds(lo, n)]

    groups = [
        [w_copy(WCH[0], 0, 256)],
        [w_copy(WCH[0], 256, D)],
        [x_copy(0, 0)],
        [x_copy(0, 1, 0, QB), w_copy(WCH[1])],
        [w_copy(WCH[2]), x_copy(0, 1, QB, QB)],
        [(wb, wv.at[1]), x_copy(1, 0), x_copy(1, 1), (woa, wov.at[0]), (wob, wov.at[1])],
        [x_copy(b, k) for k in range(2, NX) for b in range(2)],
    ]
    osem = sem.at[len(groups)]

    def in_copies(n):
        return [pltpu.make_async_copy(src, dst, sem.at[n]) for src, dst in groups[n]]

    def run(prog, it=None):
        off = 0 if it is None else it * PB
        val = {}
        pend = []

        def rows(q, n=1):
            if it is None:
                return pl.ds(q * QB, n * QB)
            return pl.ds(pl.multiple_of((q + off) * QB, QB), n * QB)

        def take_deps():
            ready = [_zero_of(c, x) for n, x in pend if n == 0]
            pend[:] = [(n - 1, x) for n, x in pend if n > 0]
            return ready

        def store_out(q, c0, c1, x):
            x = x.T.astype(BF16)
            ob[rows(q), c0:c1] = x
            pend.append((1, pltpu.bitcast(x[QB - 16:], U32)))

        for item in prog:
            op, a = item[0], item[1:]
            if op == "WAIT":
                for cp in in_copies(a[0]):
                    cp.wait()
            elif op == "TW":
                b, (lo, n), r0, r1 = a
                wt[b, lo // 2:(lo + n) // 2, r0:r1] = pltpu.bitcast(wv[b, r0:r1, lo:lo + n].T, U32)
            elif op == "TO":
                wot[a[0]] = pltpu.bitcast(wov[a[0]].T, U32)
            elif op == "K":
                pend.append((1, _prep_k(c, *a, _proj(c, *a, off, 1))))
            elif op == "KM":
                val["k", a] = _proj(c, *a, off, 1)
            elif op == "KP":
                _prep_k(c, *a, val.pop(("k", a)))
            elif op == "Q":
                qt[a[0], a[1] % 2] = _pack(_proj(c, *a, off, 0) * QSCALE)
            elif op == "V":
                _store_v(c, *a, _proj(c, *a, off, 2))
            elif op == "QK":
                val[a] = _scores(c, *a, take_deps())
            elif op == "QKS":
                _save_scores(c, _scores(c, *a, take_deps()))
            elif op == "AV":
                _softmax_pv(c, val.pop(a), *a)
            elif op == "AVL":
                _softmax_pv(c, _load_scores(c), *a)
            elif op in ("O", "OA"):
                b, q = a
                o = jnp.dot(_bf(wot[b]), _bf(ot[b, q % PB]), preferred_element_type=F32)
                if op == "OA":
                    store_out(q, 0, CA, o[0:CA])
                    val["tail"] = o[CA:]
                elif b == 0:
                    val["o", q] = o
                else:
                    store_out(q, 0, 2 * D, _cat([val.pop(("o", q)), o]))
            elif op == "OP":
                b, q, lo, hi = a
                rhs = _bf(ot[b, q % PB, lo // 2:hi // 2, :])
                cuts = (0, 32, 96, 160, 224) if lo == 0 else (0, 56, 112, 168, 224)
                part = [jnp.dot(_bf(wot[b, r0:r1, lo:hi]), rhs, preferred_element_type=F32)
                        for r0, r1 in zip(cuts, cuts[1:])]
                if "part" in val:
                    prev = _cat(val["part"])
                    part = [x + prev[2 * r0:2 * r1] for x, r0, r1 in zip(part, cuts, cuts[1:])]
                val["part"] = part
            elif op == "OE":
                store_out(a[1], CA, 2 * D, _cat([val.pop("tail")] + val.pop("part")))
            elif op == "OUT":
                r, cols = rows(a[0], a[1]), pl.ds(a[2], a[3] - a[2])
                pltpu.make_async_copy(ob.at[r, cols], out.at[0, r, cols], osem).start()
            else:
                raise ValueError(op)
        assert not val

    for n in range(len(groups)):
        for cp in in_copies(n):
            cp.start()

    def iota(rows, dim):
        return lax.broadcasted_iota(jnp.int32, (rows, QB), dim)

    def bits(mask, word=0xFFFFFFFF):
        return jnp.where(mask, jnp.uint32(word), jnp.uint32(0))

    phead = iota(HG, 0) // (DH // 2)
    sub = iota(HG, 1) // 16
    for t in range(4):
        slot = 2 * (sub // 4) + (jnp.where(sub % 4 >= t, 1, 0) if t else 0)
        for s in range(4):
            wm[t, s] = bits(phead == (slot ^ s))
    lane8, row8 = iota(8, 1), iota(8, 0)
    lane16, row16 = iota(16, 1), iota(16, 0)
    hib = bits(lane16 >= 64)
    for k in range(2):
        key = 32 * k + 2 * row16
        tb = bits(key <= lane16 % 64, 0xFFFF) | bits(key + 1 <= lane16 % 64, 0xFFFF0000)
        pm[0, k] = ~(tb | hib)
        pm[1, k] = ~(tb & hib)
        pm[2, k] = tb | hib
        pm[3, k] = tb & hib
    row64 = iota(64, 0)
    c.tri = 16 * (row64 // 16) + 2 * (row64 % 8) + (row64 // 8) % 2 <= iota(64, 1) % 64
    c.hi16 = lane16 >= 64
    c.hi64 = iota(64, 1) >= 64
    c.hodd = (lane8 // DH) % 2 == 1
    c.hhi = iota(HQ, 1) >= 2 * DH
    c.low4 = row8 < 4
    c.ones = jnp.where(row8 % 4 == 0, 1.0, 0.0).astype(F32)

    pro, body, epi = _programs()

    def step(it, carry):
        @pl.when(it == 0)
        def _():
            run(pro)

        run(body, it)

        @pl.when(it == NIT - 1)
        def _():
            run(epi)
            pltpu.make_async_copy(ob, out.at[0], osem).wait()

        return carry

    lax.fori_loop(0, NIT, step, 0)


@jax.jit
def pallas_concat_heads__sliding_block__sliding_block__prompt_kernel(
        A_x, A_wqkv, A_wo, B_x, B_wqkv, B_wo):
    xa = jnp.transpose(A_x, (0, 2, 1))
    xb = jnp.transpose(B_x, (0, 2, 1))
    return pl.pallas_call(
        _kernel,
        in_specs=[pl.BlockSpec(memory_space=pl.ANY)] * 6,
        out_specs=pl.BlockSpec(memory_space=pl.ANY),
        out_shape=jax.ShapeDtypeStruct((1, S, 2 * D), BF16),
        scratch_shapes=[
            pltpu.VMEM((2, D, 3 * D), BF16),
            pltpu.VMEM((2, D, D), BF16),
            pltpu.VMEM((2, NX, D, XCH), BF16),
            pltpu.VMEM((S, 2 * D), BF16),
            pltpu.VMEM((2, 3 * HD, D), U32),
            pltpu.VMEM((2, HD, D), U32),
            pltpu.VMEM((4, 4, HG, QB), U32),
            pltpu.VMEM((4, 2, 16, QB), U32),
            pltpu.VMEM((2, 2, HD, QB), U32),
            pltpu.VMEM((2, G, 32, QB), U32),
            pltpu.VMEM((2, PB, G, 2, HQ, QB), U32),
            pltpu.VMEM((2, PB, H * 16, QB), U32),
            pltpu.VMEM((2, PB, HD, QB), U32),
            pltpu.VMEM((4, 264, QB), F32),
            pltpu.SemaphoreType.DMA((8,)),
        ],
        compiler_params=pltpu.CompilerParams(
            vmem_limit_bytes=64 * 1024 * 1024,
            disable_semaphore_checks=True),
        name="swa_fused",
    )(xa, A_wqkv, A_wo, xb, B_wqkv, B_wo)
```

```python
import functools
import math

import jax
import jax.numpy as jnp
from jax import lax
from jax.experimental import pallas as pl
from jax.experimental.pallas import tpu as pltpu

S = 2048
D = 448
H = 16
DH = 28
G = 4
GW = 112
QB = 128
NQ = S // QB
HD = D // 2
HG = GW // 2
HQ = QB // 2
NEG = -1e30
QSCALE = (DH ** -0.5) * math.log2(math.e)

F32 = jnp.float32
BF16 = jnp.bfloat16
U32 = jnp.uint32

WCH = ((384, 512), (0, 384), (896, 448))
XCH = 256
NX = S // XCH
CA = 384
L0 = 3
PB = 6
NIT = (NQ - 1 - L0) // PB


def _pack(x):
    return pltpu.bitcast(x.astype(BF16), U32)


def _bf(x):
    return pltpu.bitcast(x, BF16)


def _cat(xs, axis=0):
    return xs[0] if len(xs) == 1 else jnp.concatenate(xs, axis=axis)


class _Refs:
    pass


def _zero_of(c, x):
    parts = [x[r:r + 8, l:l + QB] for r in range(0, x.shape[0], 8) for l in range(0, x.shape[1], QB)]
    return functools.reduce(lambda u, v: u | v, parts) & c.pm[0, 0, 0:8] & c.pm[2, 0, 0:8]


def _scores(c, b, q, g, deps=()):
    qg = c.qt[b, q % 2, g * HG:(g + 1) * HG, :]
    zero8 = jnp.zeros((8, QB), U32)
    if deps:
        z = functools.reduce(lambda u, v: u | v, deps)
        qg = _cat([qg[0:HG - 8], qg[HG - 8:] | z])

    def wmat(t, s):
        if t:
            return _bf(_cat([qg & c.wm[t, s], zero8]))
        rows, run = [], []
        for n in range(HG // 8 + 1):
            if {(16 * n) // DH, (16 * n + 15) // DH} & {s, s ^ 2}:
                run.append(n)
                continue
            if run:
                lo, hi = 8 * run[0], 8 * run[-1] + 8
                rows.append(qg[lo:hi] & c.wm[0, s, lo:hi])
            rows.append(zero8)
            run = []
        return _bf(_cat(rows))

    @functools.lru_cache(None)
    def krows(v, lo, hi):
        parts = []
        for blk in range((4 + lo) // 8, (4 + hi - 1) // 8 + 1):
            n0 = max(4 + lo - 8 * blk, 0)
            n1 = min(4 + hi - 8 * blk, 8)
            parts.append(c.ks[b, (q + blk) % PB, g, v, 8 * n0:8 * n1, :])
        return _cat(parts)

    def mm(rows, w):
        return jnp.dot(_bf(rows), w, preferred_element_type=F32)

    def mixed(t):
        res = []
        for s in range(4):
            hi, lo = krows(s // 2, t, t + 1), krows(s // 2, t - 17, t - 16)
            row = lax.select(c.hodd, lo, hi) if s % 2 else lax.select(c.hodd, hi, lo)
            res.append(mm(row, wmat(t, s)))
        return res

    scs = []
    if q >= 2:
        mix = {}
        for t in (1, 2, 0, 3):
            if t == 0:
                com = [mm(krows(s // 2, -13, 1), wmat(0, s)) for s in range(4)]
            else:
                mix[t] = mixed(t)
        for s in range(4):
            hi = _cat([com[s][208:224]] + [mix[t][s ^ 1] for t in (1, 2, 3)])
            lo = _cat([mix[t][s] for t in (1, 2, 3)] + [com[s][0:16]])
            scs.append(_cat([com[s][16:208], lax.select(c.tri, hi, lo)]))
    else:
        neg = jnp.full((64, QB), NEG, F32)
        for s in range(4):
            sc = mm(krows(s // 2, -4 - 8 * q, 4), wmat(0, s))
            scs.append(_cat([lax.select(c.hi64, sc[0:64], neg)] + ([sc[64:192]] if q else [])
                            + [lax.select(c.tri, sc[64 + 128 * q:], neg)]))
    res = []
    for sc in scs:
        mx = functools.reduce(jnp.maximum, [sc[r:r + 64] for r in range(0, sc.shape[0], 64)])
        res.append((sc, jnp.broadcast_to(jnp.max(mx, axis=0, keepdims=True), (8, QB))))
    return res


def _save_scores(c, sc):
    for s, (x, m) in enumerate(sc):
        c.sv[s] = _cat([x, m])


def _load_scores(c):
    return [(c.sv[s, 0:256], c.sv[s, 256:264]) for s in range(4)]


def _softmax_pv(c, sc, b, q, g):
    t0 = max(2 - q, 0)
    top = sc[0][0].shape[0] - 64
    mbits = [pltpu.bitcast(m, U32) for _, m in sc]
    mcur = [_cat([m] * 4) for _, m in sc]
    pm = functools.lru_cache(None)(lambda i, k: c.pm[i, k])

    @functools.lru_cache(None)
    def P(s, k):
        p = jnp.exp2(sc[s][0][top + 32 * k:top + 32 * k + 32] - mcur[s])
        p = pltpu.bitcast(p, U32).reshape(2, 16, QB)
        return ((p[:, 8:16] & jnp.uint32(0xFFFF0000)) | (p[:, 0:8] >> 16)).reshape(16, QB)

    def pt_rows(h, n):
        if n < 2:
            return P(h, n) & pm(0, n)
        if n >= 10:
            return P(h ^ 2, n - 10) & pm(3, n - 10)
        x = lax.select(c.hi16, P(h ^ 2, n - 2 if n < 4 else n - 10), P(h, n - 8))
        if n < 4:
            return x & pm(1, n - 2)
        return x & pm(2, n - 8) if n >= 8 else x

    acc = [None] * 4
    for t in range(2, t0 - 1, -1):
        dt = [[None] * 4 for _ in range(4)]
        for n in range(4 * t + 3, 4 * t - 1, -1):
            for h in range(4):
                dt[h][n - 4 * t] = pt_rows(h, n)
            if n > max(4, 4 * t0):
                for s in range(4):
                    z = dt[s ^ 3][n - 4 * t][8:16] >> 31
                    mcur[s] = _cat([pltpu.bitcast(mbits[s] | (z + z), F32)] * 4)
        for h in range(4):
            head = g * 4 + h
            vt = _bf(c.vt[b, (q - 2 + t) % PB, head * 16:(head + 1) * 16, :])
            o = jnp.dot(vt, _bf(_cat(dt[h])), preferred_element_type=F32)
            acc[h] = o if acc[h] is None else o + acc[h]
    outs = []
    for h in range(4):
        o = acc[h]
        l = o[28:29] if h % 2 == 0 else o[0:1]
        r = pl.reciprocal(l, approx=True)
        r = r * (2.0 - l * r)
        outs.append(o * r)
    res = []
    for p in range(2):
        e, o = outs[2 * p], outs[2 * p + 1]
        res += [e[0:24], lax.select(c.low4, e[24:32], o[0:8]), o[8:32]]
    c.ot[b, q % PB, g * HG:(g + 1) * HG, :] = _pack(_cat(res))


def _proj(c, b, q, off, part):
    x = c.xv[b, q // 2 + off, :, (q % 2) * QB:(q % 2 + 1) * QB]
    return jnp.dot(_bf(c.wt[b, part * HD:(part + 1) * HD, :]), x, preferred_element_type=F32)


def _prep_k(c, b, q, kT):
    zpad = jnp.zeros((16, QB), F32)
    last = []
    slabs = _cat([x for g in range(G) for x in (kT[g * GW:(g + 1) * GW], zpad)])
    kp = pltpu.bitcast(slabs.astype(BF16).T, U32)
    for g in range(G):
        w = kp[:, g * QB:(g + 1) * QB]
        ev = pltpu.bitcast(w << 16, F32)
        od = pltpu.bitcast(w & jnp.uint32(0xFFFF0000), F32)
        knew = _pack(_cat([ev.reshape(8, 8, QB), od.reshape(8, 8, QB)], axis=1).reshape(QB, QB))
        prev = jnp.zeros((32, QB), U32) if q == 0 else c.kr[b, g]
        c.kr[b, g] = knew[32:]
        lag = _cat([prev, knew[0:32]])
        c.ks[b, q % PB, g, 0] = lax.select(c.hhi, knew, lag)
        c.ks[b, q % PB, g, 1] = lax.select(c.hhi, lag, knew)
        last.append(knew[HQ - 8:])
    return _cat(last)


def _store_v(c, b, q, vT):
    rows = []
    for p in range(H // 2):
        base = 56 * p
        mid = vT[base + 24:base + 32]
        rows += [vT[base:base + 24], lax.select(c.low4, mid, c.ones),
                 lax.select(c.low4, c.ones, mid), vT[base + 32:base + 56]]
    c.vt[b, q % PB] = _pack(_cat(rows))


def _unit(b, q, fill, extra=(), sync=(), at=0):
    r = []
    for g in range(G):
        r += [("QK", b, q, g)] + (list(sync) if g == at else []) + [fill[g], ("AV", b, q, g)]
        if g < len(extra) and extra[g]:
            r.append(extra[g])
    return r


def _steady(b, q):
    return _unit(b, q, [("O", b, q - 1), ("K", b, q + 1), ("Q", b, q + 1), ("V", b, q + 1)])


def _programs():
    A, B = 0, 1
    KC, QC, VC = WCH
    pro = [("WAIT", 0), ("TW", A, KC, 0, 256), ("WAIT", 1), ("TW", A, KC, 256, D),
           ("WAIT", 2), ("KM", A, 0), ("KM", A, 1),
           ("WAIT", 3), ("TW", A, QC, 0, D), ("KP", A, 0), ("KP", A, 1), ("K", A, 2),
           ("Q", A, 0), ("Q", A, 1),
           ("WAIT", 4), ("TW", A, VC, 0, D)]
    pro += [("QK", A, 0, g) for g in range(G)] + [("V", A, 0)] + [("AV", A, 0, g) for g in range(G)]
    pro += _unit(A, 1, [("V", A, 1), ("Q", A, 2), ("V", A, 2), ("K", A, 3)])
    sync = [("WAIT", 5)] + [("TW", B, ch, 0, D) for ch in WCH] + [("TO", A), ("TO", B)]
    pro += _unit(A, 2, [("Q", A, 3), ("V", A, 3), ("K", B, 0), ("Q", B, 0)], sync=sync, at=1)
    pro += [("V", B, 0)]
    pro += _unit(B, 0, [("K", B, 1), ("Q", B, 1), ("O", A, 0), ("O", A, 1)])
    pro += _unit(B, 1, [("V", B, 1), ("K", B, 2), ("Q", B, 2), ("V", B, 2)],
                 extra=[None, ("O", B, 0)])
    pro += _steady(B, 2) + [("QKS", A, L0, 0), ("OUT", 0, L0 - 1, 0, 2 * D), ("WAIT", 6)]

    body = []
    for j in range(PB):
        body += _steady(A, L0 + j) + _steady(B, L0 + j)
    body = body[1:] + [("QKS", A, L0 + PB, 0), ("OUT", L0 - 1, PB, 0, 2 * D)]
    body[1] = ("AVL",) + body[1][1:]

    q = NQ - 1
    epi = [("O", A, q - 1), ("AVL", A, q, 0), ("QK", A, q, 1),
           ("O", B, q - 1), ("OUT", q - 1, 1, 0, 2 * D), ("AV", A, q, 1),
           ("QK", A, q, 2), ("QK", A, q, 3), ("AV", A, q, 2), ("QK", B, q, 3), ("AV", A, q, 3),
           ("QK", B, q, 2), ("AV", B, q, 3), ("OA", A, q), ("OUT", q, 1, 0, CA), ("AV", B, q, 2),
           ("QK", B, q, 1), ("QK", B, q, 0), ("AV", B, q, 1), ("OP", B, q, 256, D),
           ("AV", B, q, 0), ("OP", B, q, 128, 256), ("OP", B, q, 0, 128), ("OE", B, q)]
    return pro, body, epi


def _kernel(xa, wa, woa, xb, wb, wob, out, wv, wov, xv, ob, wt, wot, wm, pm, qt, kr, ks, vt, ot,
            sv, sem):
    c = _Refs()
    c.wt, c.wm, c.pm, c.qt, c.kr, c.ks, c.vt, c.ot, c.xv, c.sv = (
        wt, wm, pm, qt, kr, ks, vt, ot, xv, sv)

    def w_copy(ch, r0=0, r1=D):
        rows, cols = pl.ds(r0, r1 - r0), pl.ds(*ch)
        return wa.at[rows, cols], wv.at[0, rows, cols]

    def x_copy(b, k, lo=0, n=XCH):
        return (xa, xb)[b].at[0, :, pl.ds(k * XCH + lo, n)], xv.at[b, k, :, pl.ds(lo, n)]

    groups = [
        [w_copy(WCH[0], 0, 256)],
        [w_copy(WCH[0], 256, D)],
        [x_copy(0, 0)],
        [x_copy(0, 1, 0, QB), w_copy(WCH[1])],
        [w_copy(WCH[2]), x_copy(0, 1, QB, QB)],
        [(wb, wv.at[1]), x_copy(1, 0), x_copy(1, 1), (woa, wov.at[0]), (wob, wov.at[1])],
        [x_copy(b, k) for k in range(2, NX) for b in range(2)],
    ]
    osem = sem.at[len(groups)]

    def in_copies(n):
        return [pltpu.make_async_copy(src, dst, sem.at[n]) for src, dst in groups[n]]

    def run(prog, it=None):
        off = 0 if it is None else it * (PB // 2)
        val = {}
        pend = []

        def rows(q, n=1):
            if it is None:
                return pl.ds(q * QB, n * QB)
            return pl.ds(pl.multiple_of(q * QB + off * XCH, QB), n * QB)

        def take_deps():
            ready = [_zero_of(c, x) for n, x in pend if n == 0]
            pend[:] = [(n - 1, x) for n, x in pend if n > 0]
            return ready

        def store_out(q, c0, c1, x):
            x = x.T.astype(BF16)
            ob[rows(q), c0:c1] = x
            pend.append((1, pltpu.bitcast(x[QB - 16:], U32)))

        for item in prog:
            op, a = item[0], item[1:]
            if op == "WAIT":
                for cp in in_copies(a[0]):
                    cp.wait()
            elif op == "TW":
                b, (lo, n), r0, r1 = a
                wt[b, lo // 2:(lo + n) // 2, r0:r1] = pltpu.bitcast(wv[b, r0:r1, lo:lo + n].T, U32)
            elif op == "TO":
                wot[a[0]] = pltpu.bitcast(wov[a[0]].T, U32)
            elif op == "K":
                pend.append((1, _prep_k(c, *a, _proj(c, *a, off, 1))))
            elif op == "KM":
                val["k", a] = _proj(c, *a, off, 1)
            elif op == "KP":
                _prep_k(c, *a, val.pop(("k", a)))
            elif op == "Q":
                qt[a[0], a[1] % 2] = _pack(_proj(c, *a, off, 0) * QSCALE)
            elif op == "V":
                _store_v(c, *a, _proj(c, *a, off, 2))
            elif op == "QK":
                val[a] = _scores(c, *a, take_deps())
            elif op == "QKS":
                _save_scores(c, _scores(c, *a, take_deps()))
            elif op == "AV":
                _softmax_pv(c, val.pop(a), *a)
            elif op == "AVL":
                _softmax_pv(c, _load_scores(c), *a)
            elif op in ("O", "OA"):
                b, q = a
                o = jnp.dot(_bf(wot[b]), _bf(ot[b, q % PB]), preferred_element_type=F32)
                if op == "OA":
                    store_out(q, 0, CA, o[0:CA])
                    val["tail"] = o[CA:]
                elif b == 0:
                    val["o", q] = o
                else:
                    store_out(q, 0, 2 * D, _cat([val.pop(("o", q)), o]))
            elif op == "OP":
                b, q, lo, hi = a
                rhs = _bf(ot[b, q % PB, lo // 2:hi // 2, :])
                cuts = (0, 32, 96, 160, 224) if lo == 0 else (0, 56, 112, 168, 224)
                part = [jnp.dot(_bf(wot[b, r0:r1, lo:hi]), rhs, preferred_element_type=F32)
                        for r0, r1 in zip(cuts, cuts[1:])]
                if "part" in val:
                    prev = _cat(val["part"])
                    part = [x + prev[2 * r0:2 * r1] for x, r0, r1 in zip(part, cuts, cuts[1:])]
                val["part"] = part
            elif op == "OE":
                x = _cat([val.pop("tail")] + val.pop("part")).T.astype(BF16)
                n = 16
                for k in range(QB // n):
                    r = pl.ds(a[1] * QB + k * n, n)
                    ob[r, CA:] = x[k * n:(k + 1) * n]
                    pltpu.make_async_copy(ob.at[r, pl.ds(CA, 2 * D - CA)],
                                          out.at[0, r, pl.ds(CA, 2 * D - CA)], osem).start()
            elif op == "OUT":
                r, cols = rows(a[0], a[1]), pl.ds(a[2], a[3] - a[2])
                pltpu.make_async_copy(ob.at[r, cols], out.at[0, r, cols], osem).start()
            else:
                raise ValueError(op)
        assert not val

    for n in range(len(groups)):
        for cp in in_copies(n):
            cp.start()

    def iota(rows, dim):
        return lax.broadcasted_iota(jnp.int32, (rows, QB), dim)

    def bits(mask, word=0xFFFFFFFF):
        return jnp.where(mask, jnp.uint32(word), jnp.uint32(0))

    phead = iota(HG, 0) // (DH // 2)
    sub = iota(HG, 1) // 16
    for t in range(4):
        slot = 2 * (sub // 4) + (jnp.where(sub % 4 >= t, 1, 0) if t else 0)
        for s in range(4):
            wm[t, s] = bits(phead == (slot ^ s))
    lane8, row8 = iota(8, 1), iota(8, 0)
    lane16, row16 = iota(16, 1), iota(16, 0)
    hib = bits(lane16 >= 64)
    for k in range(2):
        key = 32 * k + 2 * row16
        tb = bits(key <= lane16 % 64, 0xFFFF) | bits(key + 1 <= lane16 % 64, 0xFFFF0000)
        pm[0, k] = ~(tb | hib)
        pm[1, k] = ~(tb & hib)
        pm[2, k] = tb | hib
        pm[3, k] = tb & hib
    row64 = iota(64, 0)
    c.tri = 16 * (row64 // 16) + 2 * (row64 % 8) + (row64 // 8) % 2 <= iota(64, 1) % 64
    c.hi16 = lane16 >= 64
    c.hi64 = iota(64, 1) >= 64
    c.hodd = (lane8 // DH) % 2 == 1
    c.hhi = iota(HQ, 1) >= 2 * DH
    c.low4 = row8 < 4
    c.ones = jnp.where(row8 % 4 == 0, 1.0, 0.0).astype(F32)

    pro, body, epi = _programs()

    def step(it, carry):
        @pl.when(it == 0)
        def _():
            run(pro)

        run(body, it)

        @pl.when(it == NIT - 1)
        def _():
            run(epi)
            pltpu.make_async_copy(ob, out.at[0], osem).wait()

        return carry

    lax.fori_loop(0, NIT, step, 0)


@jax.jit
def pallas_concat_heads__sliding_block__sliding_block__prompt_kernel(
        A_x, A_wqkv, A_wo, B_x, B_wqkv, B_wo):
    xa = jnp.transpose(A_x, (0, 2, 1))
    xb = jnp.transpose(B_x, (0, 2, 1))
    return pl.pallas_call(
        _kernel,
        in_specs=[pl.BlockSpec(memory_space=pl.ANY)] * 6,
        out_specs=pl.BlockSpec(memory_space=pl.ANY),
        out_shape=jax.ShapeDtypeStruct((1, S, 2 * D), BF16),
        scratch_shapes=[
            pltpu.VMEM((2, D, 3 * D), BF16),
            pltpu.VMEM((2, D, D), BF16),
            pltpu.VMEM((2, NX, D, XCH), BF16),
            pltpu.VMEM((S, 2 * D), BF16),
            pltpu.VMEM((2, 3 * HD, D), U32),
            pltpu.VMEM((2, HD, D), U32),
            pltpu.VMEM((4, 4, HG, QB), U32),
            pltpu.VMEM((4, 2, 16, QB), U32),
            pltpu.VMEM((2, 2, HD, QB), U32),
            pltpu.VMEM((2, G, 32, QB), U32),
            pltpu.VMEM((2, PB, G, 2, HQ, QB), U32),
            pltpu.VMEM((2, PB, H * 16, QB), U32),
            pltpu.VMEM((2, PB, HD, QB), U32),
            pltpu.VMEM((4, 264, QB), F32),
            pltpu.SemaphoreType.DMA((8,)),
        ],
        compiler_params=pltpu.CompilerParams(
            vmem_limit_bytes=64 * 1024 * 1024,
            disable_semaphore_checks=True),
        name="swa_fused",
    )(xa, A_wqkv, A_wo, xb, B_wqkv, B_wo)
```
